```python
import os as _os
_os.environ.setdefault("JAX_PLATFORMS", "cpu")
import jax
import jax.numpy as jnp

def _softmax(x, axis=-1):
    return jax.nn.softmax(x, axis=axis)
def _gelu(x):
    return jax.nn.gelu(x, approximate=True)
def _silu(x):
    return jax.nn.silu(x)
def _sigmoid(x):
    return jax.nn.sigmoid(x)
def _layernorm(x, axis=-1, eps=1e-5):
    m = jnp.mean(x, axis=axis, keepdims=True)
    v = jnp.var(x, axis=axis, keepdims=True)
    return (x - m) / jnp.sqrt(v + eps)
def _scatter_add(tgt, idx, src, axis=0):
    return tgt.at[idx].add(src)
def _segment_sum(src, seg, n):
    return jax.ops.segment_sum(src, seg, n)
class _Rng:
    def __init__(self, key):
        self._k = key
    def _next(self):
        self._k, sub = jax.random.split(self._k)
        return sub
    def normal(self, shape):
        return jax.random.normal(self._next(), shape, dtype=jnp.bfloat16)
    def randint(self, lo, hi, shape):
        return jax.random.randint(self._next(), shape, lo, hi, dtype=jnp.int32)
    def uniform(self, shape, lo=0.0, hi=1.0):
        return jax.random.uniform(self._next(), shape, jnp.bfloat16, lo, hi)
    def permutation(self, n):
        return jax.random.permutation(self._next(), n)


kernel_name = 'standalone__mha_block_cached__near_ridge'

def setup_inputs():
    _rng = _Rng(jax.random.key(int.from_bytes(__import__("os").urandom(4), "little")))
    _w = (lambda a: (lambda t: t.astype(jnp.bfloat16) if jnp.issubdtype(t.dtype, jnp.floating) else t)(jnp.asarray(a)))
    B, Sq, D = 8, 144, 448
    H, Sk, Dh = 16, 2048, 256
    return {
        "x": _w((lambda *s: _rng.normal(s) * 0.8)(B, Sq, D)),
        "k_cache": _w((lambda *s: _rng.normal(s) * 0.8)(B, H, Sk, Dh)),
        "v_cache": _w((lambda *s: _rng.normal(s) * 0.05)(B, H, Sk, Dh)),
        "wq": _w((lambda *s: _rng.normal(s) * 0.8)(D, H * Dh) * (D ** -0.5)),
        "wo": _w((lambda *s: _rng.normal(s) * 0.05)(H * Dh, D) * ((H * Dh) ** -0.5)),
    }

def reference(x, k_cache, v_cache, wq, wo):
    B, Sq, D = x.shape
    H, Dh = 16, 256
    q = (lambda x, *d: x.transpose(*d))((x @ wq).reshape(B, Sq, H, Dh), 0, 2, 1, 3)
    scores = jnp.einsum("bhqd,bhkd->bhqk", q, k_cache) * (Dh ** -0.5)
    p = _softmax(scores, axis=-1)
    o = jnp.einsum("bhqk,bhkd->bhqd", p, v_cache)
    return (lambda x, *d: x.transpose(*d))(o, 0, 2, 1, 3).reshape(B, Sq, H * Dh) @ wo
```

```python
import functools, math
import jax
import jax.numpy as jnp
from jax import lax
import jax.experimental.pallas as pl
import jax.experimental.pallas.tpu as pltpu

CH = 64
NT = (((1,), (1,)), ((), ()))

def diag_order(G, sub, run=2, nch=32):
    part = nch // G
    out = []
    for j in range(nch):
        r = (j // run) % G
        k = (j // (run * G)) * run + j % run
        blk = k // run
        s = blk % sub
        within = (blk // sub) * run + k % run
        out.append((r, s * (nch // sub) + r * (part // sub) + within))
    assert sorted(c for _, c in out) == list(range(nch))
    return out

def make(G=2, sub=2, KB=256, NS=8, LK=2, LV=2, semchk=True, defer=True):
    def f(x, k_cache, v_cache, wq, wo):
        B, Sq, D = x.shape
        _, H, Sk, Dh = k_cache.shape
        NH = B * H
        nch = Sk // CH
        order = diag_order(G, sub, nch=nch)
        assert NS >= max(LK, LV) + G
        nkb = Sk // KB
        qscale = (Dh ** -0.5) * math.log2(math.e)
        k3 = k_cache.reshape(NH * nch, CH, Dh)
        v3 = v_cache.reshape(NH * nch, CH, Dh)
        x2 = x.reshape(B * Sq, D)
        wot = wo.T

        def kern(x_hbm, k_hbm, v_hbm, wq_hbm, wo_hbm, out_hbm,
                 xb, wqb, wob, kb, vb, sb, qb, ob, acc, outb, semk, semv, semw, semo):
            def chunk(src, buf, sem, h, c):
                s = h & (NS - 1)
                return pltpu.make_async_copy(src.at[h * nch + c], buf.at[s, pl.ds(c * CH, CH)], sem.at[s])
            def burst(g):
                for r, c in order:
                    for prio, (src, buf, sem, lead) in enumerate(((k_hbm, kb, semk, LK), (v_hbm, vb, semv, LV))):
                        h = g + lead + r
                        if isinstance(h, int) and not 0 <= h < NH:
                            continue
                        chunk(src, buf, sem, h, c).start(priority=prio)
            def wait_item(buf, sem, g):
                s = g & (NS - 1)
                pltpu.make_async_copy(buf.at[s], buf.at[s], sem.at[s]).wait()

            nrt = D // 8
            rows = [((j // 1) % 7) * 8 + j // 7 for j in range(nrt)]
            for j, rt in enumerate(rows):
                for half in range(2):
                    for prio, (src, dst, si) in enumerate(((wq_hbm, wqb, 0), (wo_hbm, wob, 1))):
                        idx = (pl.ds(rt * 8, 8), pl.ds(half * 2048, 2048))
                        pltpu.make_async_copy(src.at[idx], dst.at[idx], semw.at[si]).start(priority=prio)
            for j in range(B * Sq // 32):
                idx = (pl.ds(j * 32, 32),)
                pltpu.make_async_copy(x_hbm.at[idx], xb.at[idx], semw.at[2]).start(priority=j % 2)
            first = -(max(LK, LV) + G - 1)
            for g in range(first, 0):
                burst(g)
            for dst, si in ((wqb, 0), (wob, 1), (xb, 2)):
                pltpu.make_async_copy(dst, dst, semw.at[si]).wait()

            def qproj(g):
                b = g // H if isinstance(g, int) else lax.shift_right_logical(g, 4)
                h = g % H if isinstance(g, int) else g & (H - 1)
                w = wqb[:, pl.ds(pl.multiple_of(h * Dh, Dh), Dh)]
                xx = xb[pl.ds(pl.multiple_of(b * Sq, 16), Sq), :]
                q = jnp.dot(xx, w, preferred_element_type=jnp.float32)
                return (q * qscale).astype(jnp.bfloat16)

            def outproj(g):
                h = g % H if isinstance(g, int) else g & (H - 1)
                w = wob[:, pl.ds(pl.multiple_of(h * Dh, Dh), Dh)]
                return lax.dot_general(ob[...], w, NT, preferred_element_type=jnp.float32)

            nmain = NH - max(LK, LV) - G + 1
            def body(g, _):
                s = g & (NS - 1)
                wait_item(kb, semk, g)
                @pl.when(g < nmain)
                def _():
                    burst(g)
                @pl.when(g >= nmain)
                def _():
                    for gg in range(nmain, NH - min(LK, LV)):
                        pl.when(g == gg)(functools.partial(burst, gg))
                q = qb[...]
                m = None
                for t in range(nkb):
                    st = lax.dot_general(q, kb[s, pl.ds(t * KB, KB), :], NT, preferred_element_type=jnp.float32)
                    sb[:, pl.ds(t * KB, KB)] = st
                    for u in range(KB // 128):
                        su = st[:, u * 128:(u + 1) * 128]
                        m = su if m is None else jnp.maximum(m, su)
                m = jnp.max(m, axis=-1, keepdims=True)
                qb[...] = qproj(jnp.minimum(g + 1, NH - 1))
                y = outproj(g - 1)
                fresh = ((g - 1) & (H - 1)) == 0
                acc[...] = jnp.where(fresh, y, acc[...] + y)
                wait_item(vb, semv, g)
                o = None; l = None
                for t in range(nkb):
                    p = jnp.exp2(sb[:, pl.ds(t * KB, KB)] - m)
                    for u in range(KB // 128):
                        pu = p[:, u * 128:(u + 1) * 128]
                        l = pu if l is None else l + pu
                    ot = jnp.dot(p.astype(jnp.bfloat16), vb[s, pl.ds(t * KB, KB), :], preferred_element_type=jnp.float32)
                    o = ot if o is None else o + ot
                l = jnp.sum(l, axis=-1, keepdims=True)
                ob[...] = (o * (1.0 / l)).astype(jnp.bfloat16)

                @pl.when(jnp.logical_and((g & (H - 1)) == 0, g > 0))
                def _():
                    b = lax.shift_right_logical(g, 4) - 1
                    outb[pl.ds(pl.multiple_of(b * Sq, 16), Sq), :] = acc[...].astype(jnp.bfloat16)

                if defer:
                    @pl.when(g == NH - 1 - min(LK, LV))
                    def _():
                        for j in range((B - 1) * Sq // 48):
                            idx = (pl.ds(j * 48, 48),)
                            pltpu.make_async_copy(outb.at[idx], out_hbm.at[idx], semo.at[0]).start(priority=1)
                return 0

            qb[...] = qproj(0)
            acc[...] = jnp.zeros_like(acc)
            ob[...] = jnp.zeros_like(ob)
            lax.fori_loop(0, NH, body, 0)
            last = pl.ds((B - 1) * Sq, Sq)
            outb[last, :] = (acc[...] + outproj(NH - 1)).astype(jnp.bfloat16)
            if defer:
                co = pltpu.make_async_copy(outb.at[last], out_hbm.at[last], semo.at[1])
                co.start()
                rest = outb.at[pl.ds(0, (B - 1) * Sq)]
                pltpu.make_async_copy(rest, rest, semo.at[0]).wait()
                co.wait()
            else:
                co = pltpu.make_async_copy(outb, out_hbm, semo.at[1])
                co.start(); co.wait()

        hbm = pl.BlockSpec(memory_space=pltpu.HBM)
        out = pl.pallas_call(
            kern,
            in_specs=[hbm] * 5,
            out_specs=hbm,
            out_shape=jax.ShapeDtypeStruct((B * Sq, D), x.dtype),
            scratch_shapes=[
                pltpu.VMEM((B * Sq, D), jnp.bfloat16),
                pltpu.VMEM((D, H * Dh), jnp.bfloat16),
                pltpu.VMEM((D, H * Dh), jnp.bfloat16),
                pltpu.VMEM((NS, Sk, Dh), jnp.bfloat16),
                pltpu.VMEM((NS, Sk, Dh), jnp.bfloat16),
                pltpu.VMEM((Sq, Sk), jnp.float32),
                pltpu.VMEM((Sq, Dh), jnp.bfloat16),
                pltpu.VMEM((Sq, Dh), jnp.bfloat16),
                pltpu.VMEM((Sq, D), jnp.float32),
                pltpu.VMEM((B * Sq, D), jnp.bfloat16),
                pltpu.SemaphoreType.DMA((NS,)),
                pltpu.SemaphoreType.DMA((NS,)),
                pltpu.SemaphoreType.DMA((3,)),
                pltpu.SemaphoreType.DMA((2,)),
            ],
            compiler_params=pltpu.CompilerParams(vmem_limit_bytes=100 * 1024 * 1024, disable_bounds_checks=True,
                                                 disable_semaphore_checks=not semchk),
        )(x2, k3, v3, wq, wot)
        return out.reshape(B, Sq, D)
    return f


@jax.jit
def pallas_standalone__mha_block_cached__near_ridge_kernel(x, k_cache, v_cache, wq, wo):
    return make(2, 2, LK=1, LV=2)(x, k_cache, v_cache, wq, wo)
```

```python
import functools, math, contextlib
import jax
import jax.numpy as jnp
from jax import lax
import jax.experimental.pallas as pl
import jax.experimental.pallas.tpu as pltpu

NT = (((1,), (1,)), ((), ()))
SR = 32
LANES = 4
DEPTH = 4
PAIR, SINGLE = 1, 2


def build_bursts(NH, Sk, n4, n2, n1):
    J = (NH - n4 - n2 - n1) // 2
    assert 2 * J + n4 + n2 + n1 == NH and n4 % 2 == 0
    J2 = J + n4 // 2
    J1 = J2 + n2
    JE = J1 + 2 * n1
    def lane(t, a):
        j = (t >> 4) - 3 + a
        if j < 0:
            return None
        if j < J:
            return (PAIR, 2 * j, (t & 63) * SR)
        if a < 2:
            return (SINGLE, 2 * j + 2, (t & 31) * SR) if j < J2 else None
        if j >= JE or (j >= J1 and (j - J1) % 2):
            return None
        return (SINGLE, min(max(j + J, 2 * j - 1), j + J2, (j + J1) // 2 + J2), (t & 31) * SR)
    bursts = []
    t = 0
    while t < 16 * JE:
        act = [d for d in (lane(t, a) for a in range(LANES)) if d]
        n = len(act)
        if n > 2 or t < 48:
            bursts.append((SR, [lane(t, a) for a in range(LANES)]))
            t += DEPTH
        else:
            r = LANES // n
            bursts.append((r * SR, [(k, h, row + i * SR) for i in range(r) for k, h, row in act]))
            t += DEPTH * r
    seen = {}
    done = {}
    for b, (step, lanes) in enumerate(bursts):
        for d in lanes:
            if d is None:
                continue
            kind, h, row = d
            for k in range(DEPTH):
                r = row + k * step
                assert r + SR <= (Sk if kind == PAIR else Sk // 2)
                for p in ([(h, r), (h + 1, r)] if kind == PAIR else [(h, r), (h, r + Sk // 2)]):
                    assert p not in seen, (b, p)
                    seen[p] = b
                    done[p[0]] = b + 1
    assert len(seen) == NH * (Sk // SR) and sorted(done) == list(range(NH))
    return bursts, [done[h] for h in range(NH)], J


def make(KB=256, NS=16, semchk=False, n4=16, n2=6, n1=4, vlead=1, lead=1, lead2=0.5, c_model=0.865,
         defer_norm=True, scoped=False, n_mid=128, flags=None, g_out=None,
         dB=(2, 2, 2, 2, 2, 2, 2, 2), dD=(2, 2, 2, 2, 2, 2, 2, 2), st_at=-1):
    def f(x, k_cache, v_cache, wq, wo):
        B, Sq, D = x.shape
        _, H, Sk, Dh = k_cache.shape
        NH = B * H
        nkb = Sk // KB
        qscale = (Dh ** -0.5) * math.log2(math.e)
        k3 = k_cache.reshape(NH, Sk, Dh)
        v3 = v_cache.reshape(NH, Sk, Dh)
        x2 = x.reshape(B * Sq, D)
        wot = wo.T
        bursts, done, J = build_bursts(NH, Sk, n4, n2, n1)
        NB = len(bursts)
        n_pair_heads = 2 * J
        need = [0] * (NH + 1)
        for g in reversed(range(NH)):
            need[g] = max(done[g] + lead, need[g + 1] - 2)
        nus = [need[0]]; skips = []
        now = done[0]
        for g in range(NH):
            now = max(now + 2 * c_model, done[min(g + 1, NH - 1)])
            if nus[-1] + 1 >= max(need[g + 1], now + lead2):
                skips.append(g); nus.append(nus[-1] + 1)
            else:
                nus.append(nus[-1] + 2)
            assert nus[g] >= done[g], (g, nus[g], done[g])
            for b in range(nus[g], min(nus[g + 1] + vlead, NB)):
                for d in bursts[b][1]:
                    assert d is None or d[1] + (d[0] == PAIR) - NS < g
        assert nus[NH] >= NB
        last_issue = max(g for g in range(NH) if nus[g] < NB)
        skips = [g for g in skips if g <= last_issue]
        go = g_out if g_out is not None else last_issue
        assert go > NH - H
        def word(step, d):
            return 0 if d is None else (d[0] << 28) | ((step // SR) << 20) | (d[1] << 11) | d[2]
        words = [[word(step, d) for d in lanes] for step, lanes in bursts]
        NT_ = nus[NH] + vlead + 1
        words += [[0] * LANES] * (NT_ - NB)
        regular = lambda b, i: (PAIR << 28) | (1 << 20) | (((b >> 2) - 3 + i) << 12) | ((b & 15) << 7)
        b_lo = 12
        b_hi = next(b for b in range(b_lo, NB) if words[b] != [regular(b, i) for i in range(LANES)])
        f.info = dict(NB=NB, last_issue=last_issue, skips=skips, b_hi=b_hi, ahead=[nus[g] - done[g] for g in range(n_pair_heads - 8, NH)])

        def kern(x_hbm, k_hbm, v_hbm, wq_hbm, wo_hbm, out_hbm,
                 xb, wqb, wob, kvb, sb, qb, ob, lb, acc, outb, tab, semkv, semw, semo):
            def start_desc(tt, kind, w, k):
                src = (k_hbm, v_hbm)[tt]
                dst = kvb.at[tt]
                h = lax.shift_right_logical(w, 11) & (NH - 1)
                s = h & (NS - 1)
                row = (w & (Sk - 1)) + k * SR * (lax.shift_right_logical(w, 20) & 7)
                rows = pl.ds(pl.multiple_of(row, SR), SR)
                if kind == PAIR:
                    c = pltpu.make_async_copy(src.at[pl.ds(h, 2), rows], dst.at[pl.ds(s, 2), rows], semkv.at[tt, s])
                else:
                    c = pltpu.make_async_copy(src.reshape(2 * NH, Sk // 2, Dh).at[pl.ds(2 * h, 2), rows],
                                              dst.reshape(2 * NS, Sk // 2, Dh).at[pl.ds(2 * s, 2), rows], semkv.at[tt, s])
                c.start(priority=tt)
            def wait_item(tt, g):
                s = g & (NS - 1)
                @pl.when(jnp.logical_and(g < n_pair_heads, (g & 1) == 0))
                def _():
                    d = kvb.at[tt, pl.ds(s, 2)]
                    pltpu.make_async_copy(d, d, semkv.at[tt, s]).wait()
                @pl.when(g >= n_pair_heads)
                def _():
                    d = kvb.at[tt, s]
                    pltpu.make_async_copy(d, d, semkv.at[tt, s]).wait()

            nrt = D // 8
            def wloop(j, _):
                rt = lax.rem(j, 7) * 4 + lax.div(j, 7)
                for quarter in range(4):
                    for prio, (src, dst, si) in enumerate(((wq_hbm, wqb, 0), (wo_hbm, wob, 1))):
                        idx = (slice(None), pl.ds(pl.multiple_of(rt * 8, 8), 8), pl.ds(quarter * 1024, 1024))
                        pltpu.make_async_copy(src.reshape(2, D // 2, H * Dh).at[idx], dst.reshape(2, D // 2, H * Dh).at[idx],
                                              semw.at[si]).start(priority=prio)
                return 0
            lax.fori_loop(0, nrt // 2, wloop, 0)
            def tloop(b, _):
                for i in range(LANES):
                    tab[LANES * b + i] = regular(b, i)
                return 0
            lax.fori_loop(b_lo, b_hi, tloop, 0)
            def xloop(j, _):
                for half in range(2):
                    idx = (slice(None), pl.ds(pl.multiple_of(j * 16 + half * (B * Sq // 4), 16), 16))
                    pltpu.make_async_copy(x_hbm.reshape(2, B * Sq // 2, D).at[idx], xb.reshape(2, B * Sq // 2, D).at[idx],
                                          semw.at[2]).start(priority=half)
                return 0
            lax.fori_loop(0, B * Sq // 64, xloop, 0)
            for b in list(range(b_lo)) + list(range(b_hi, NT_)):
                for i in range(LANES):
                    tab[LANES * b + i] = jnp.int32(words[b][i])
            def kvloop(i, _):
                for k in range(DEPTH):
                    for ln in range(LANES):
                        for tt in range(2):
                            w = tab[LANES * (i if tt else jnp.maximum(i - vlead, 0)) + ln]
                            ok = w != 0
                            if not tt:
                                ok = jnp.logical_and(ok, i >= vlead)
                            pl.when(ok)(functools.partial(start_desc, tt, PAIR, w, k))
                return 0
            assert nus[0] + vlead <= b_hi
            lax.fori_loop(0, nus[0] + vlead, kvloop, 0)
            for dst, si in ((wqb, 0), (wob, 1), (xb, 2)):
                pltpu.make_async_copy(dst, dst, semw.at[si]).wait()

            def qproj(g):
                b = g // H if isinstance(g, int) else lax.shift_right_logical(g, 4)
                h = g % H if isinstance(g, int) else g & (H - 1)
                w = wqb[:, pl.ds(pl.multiple_of(h * Dh, Dh), Dh)]
                xx = xb[pl.ds(pl.multiple_of(b * Sq, 16), Sq), :]
                q = jnp.dot(xx, w, preferred_element_type=jnp.float32)
                return (q * qscale).astype(jnp.bfloat16)

            def outproj(g):
                h = g % H if isinstance(g, int) else g & (H - 1)
                w = wob[:, pl.ds(pl.multiple_of(h * Dh, Dh), Dh)]
                if defer_norm:
                    l = jnp.sum(lb[...], axis=-1, keepdims=True)
                    o = (ob[...] * (1.0 / l)).astype(jnp.bfloat16)
                else:
                    o = ob[...]
                return lax.dot_general(o, w, NT, preferred_element_type=jnp.float32)

            def body(g, b0, midwait):
                s = g & (NS - 1)
                second = functools.reduce(jnp.logical_and, [g != sk for sk in skips], g >= 0)
                par = {}
                def dma(i0, i1):
                    for i in range(i0, i1):
                        half, k, ln = i // (LANES * DEPTH), (i // LANES) % DEPTH, i % LANES
                        for tt in range(2):
                            key = (half, tt, ln)
                            if key not in par:
                                w = tab[LANES * b0 + (LANES * (half + (vlead if tt else 0)) + ln)]
                                if half:
                                    w = jnp.where(second, w, 0)
                                par[key] = w
                            w = par[key]
                            for kind in (PAIR, SINGLE):
                                pl.when(lax.shift_right_logical(w, 28) == kind)(functools.partial(start_desc, tt, kind, w, k))
                cuts = [0]
                for c_ in tuple(dB) + tuple(dD):
                    cuts.append(cuts[-1] + c_)
                assert cuts[-1] == 2 * LANES * DEPTH and len(cuts) == 2 * nkb + 1
                with (jax.named_scope("wk") if scoped else contextlib.nullcontext()):
                    wait_item(0, g)
                if not midwait:
                    wait_item(1, g)
                q = qb[...]
                m = None
                for t in range(nkb):
                    kt = kvb[0, s, pl.ds(t * KB, KB), :]
                    dma(cuts[t], cuts[t + 1])
                    st = lax.dot_general(q, kt, NT, preferred_element_type=jnp.float32)
                    sb[:, pl.ds(t * KB, KB)] = st
                    for u in range(KB // 128):
                        su = st[:, u * 128:(u + 1) * 128]
                        m = su if m is None else jnp.maximum(m, su)
                m = jnp.max(m, axis=-1, keepdims=True)
                qn = qproj(jnp.minimum(g + 1, NH - 1))
                y = outproj(g - 1)
                def store_proj():
                    qb[...] = qn
                    fresh = ((g - 1) & (H - 1)) == 0
                    acc[...] = jnp.where(fresh, y, acc[...] + y)
                if st_at < 0:
                    store_proj()
                if midwait:
                    with (jax.named_scope("wv") if scoped else contextlib.nullcontext()):
                        wait_item(1, g)
                o = None; l = None
                for t in range(nkb):
                    vt = kvb[1, s, pl.ds(t * KB, KB), :]
                    dma(cuts[nkb + t], cuts[nkb + t + 1])
                    p = jnp.exp2(sb[:, pl.ds(t * KB, KB)] - m)
                    for u in range(KB // 128):
                        pu = p[:, u * 128:(u + 1) * 128]
                        l = pu if l is None else l + pu
                    ot = jnp.dot(p.astype(jnp.bfloat16), vt, preferred_element_type=jnp.float32)
                    o = ot if o is None else o + ot
                    if t == st_at:
                        store_proj()
                if defer_norm:
                    ob[...] = o
                    lb[...] = l
                else:
                    l = jnp.sum(l, axis=-1, keepdims=True)
                    ob[...] = (o * (1.0 / l)).astype(jnp.bfloat16)

                @pl.when(jnp.logical_and((g & (H - 1)) == 0, g > 0))
                def _():
                    b = lax.shift_right_logical(jnp.maximum(g - 1, 0), 4)
                    outb[pl.ds(pl.multiple_of(b * Sq, 16), Sq), :] = acc[...].astype(jnp.bfloat16)

                @pl.when(g == go)
                def _():
                    n = (B - 1) * Sq
                    def wr(j, _):
                        for half in range(2):
                            r = pl.ds(pl.multiple_of(half * (n // 2) + j * 24, 8), 24)
                            pltpu.make_async_copy(outb.at[r], out_hbm.at[r], semo.at[0]).start(priority=1)
                        return 0
                    lax.fori_loop(0, n // 2 // 24, wr, 0)
                return b0 + 1 + second.astype(jnp.int32)

            qb[...] = qproj(0)
            acc[...] = jnp.zeros_like(acc)
            ob[...] = jnp.zeros_like(ob)
            lb[...] = jnp.ones_like(lb)
            def sbody(g, c, midwait):
                with (jax.named_scope("it") if scoped else contextlib.nullcontext()):
                    return body(g, c, midwait)
            bb = nus[0]
            if n_mid < NH:
                bb = lax.fori_loop(0, NH - n_mid, functools.partial(sbody, midwait=False), bb)
            if n_mid > 0:
                lax.fori_loop(NH - n_mid, NH, functools.partial(sbody, midwait=True), bb)
            last = pl.ds((B - 1) * Sq, Sq)
            outb[last, :] = (acc[...] + outproj(NH - 1)).astype(jnp.bfloat16)
            co = pltpu.make_async_copy(outb.at[last], out_hbm.at[last], semo.at[1])
            co.start()
            rest = outb.at[pl.ds(0, (B - 1) * Sq)]
            with (jax.named_scope("wo1") if scoped else contextlib.nullcontext()):
                pltpu.make_async_copy(rest, rest, semo.at[0]).wait()
            with (jax.named_scope("wo2") if scoped else contextlib.nullcontext()):
                co.wait()

        hbm = pl.BlockSpec(memory_space=pltpu.HBM)
        out = pl.pallas_call(
            kern,
            in_specs=[hbm] * 5,
            out_specs=hbm,
            out_shape=jax.ShapeDtypeStruct((B * Sq, D), x.dtype),
            scratch_shapes=[
                pltpu.VMEM((B * Sq, D), jnp.bfloat16),
                pltpu.VMEM((D, H * Dh), jnp.bfloat16),
                pltpu.VMEM((D, H * Dh), jnp.bfloat16),
                pltpu.VMEM((2, NS, Sk, Dh), jnp.bfloat16),
                pltpu.VMEM((Sq, Sk), jnp.float32),
                pltpu.VMEM((Sq, Dh), jnp.bfloat16),
                pltpu.VMEM((Sq, Dh), jnp.float32 if defer_norm else jnp.bfloat16),
                pltpu.VMEM((Sq, 128), jnp.float32),
                pltpu.VMEM((Sq, D), jnp.float32),
                pltpu.VMEM((B * Sq, D), jnp.bfloat16),
                pltpu.SMEM((NT_ * LANES,), jnp.int32),
                pltpu.SemaphoreType.DMA((2, NS)),
                pltpu.SemaphoreType.DMA((3,)),
                pltpu.SemaphoreType.DMA((2,)),
            ],
            compiler_params=pltpu.CompilerParams(vmem_limit_bytes=100 * 1024 * 1024, disable_bounds_checks=True,
                                                 disable_semaphore_checks=not semchk, flags=flags),
        )(x2, k3, v3, wq, wot)
        return out.reshape(B, Sq, D)
    return f


@jax.jit
def pallas_standalone__mha_block_cached__near_ridge_kernel(x, k_cache, v_cache, wq, wo):
    return make(n4=20,n2=8,n1=6,lead2=1)(x, k_cache, v_cache, wq, wo)
```

```python
import functools, math, contextlib
import jax
import jax.numpy as jnp
from jax import lax
import jax.experimental.pallas as pl
import jax.experimental.pallas.tpu as pltpu

NT = (((1,), (1,)), ((), ()))
SR = 32
LANES = 4
DEPTH = 4
PAIR, SINGLE = 1, 2


def build_bursts(NH, Sk, n4, n2, n1):
    J = (NH - n4 - n2 - n1) // 2
    assert 2 * J + n4 + n2 + n1 == NH and n4 % 2 == 0
    J2 = J + n4 // 2
    J1 = J2 + n2
    JE = J1 + 2 * n1
    def lane(t, a):
        j = (t >> 4) - 3 + a
        if j < 0:
            return None
        if j < J:
            return (PAIR, 2 * j, (t & 63) * SR)
        if a < 2:
            return (SINGLE, 2 * j + 2, (t & 31) * SR) if j < J2 else None
        if j >= JE or (j >= J1 and (j - J1) % 2):
            return None
        return (SINGLE, min(max(j + J, 2 * j - 1), j + J2, (j + J1) // 2 + J2), (t & 31) * SR)
    bursts = []
    t = 0
    while t < 16 * JE:
        act = [d for d in (lane(t, a) for a in range(LANES)) if d]
        n = len(act)
        if n > 2 or t < 48:
            bursts.append((SR, [lane(t, a) for a in range(LANES)]))
            t += DEPTH
        else:
            r = LANES // n
            bursts.append((r * SR, [(k, h, row + i * SR) for i in range(r) for k, h, row in act]))
            t += DEPTH * r
    seen = {}
    done = {}
    for b, (step, lanes) in enumerate(bursts):
        for d in lanes:
            if d is None:
                continue
            kind, h, row = d
            for k in range(DEPTH):
                r = row + k * step
                assert r + SR <= (Sk if kind == PAIR else Sk // 2)
                for p in ([(h, r), (h + 1, r)] if kind == PAIR else [(h, r), (h, r + Sk // 2)]):
                    assert p not in seen, (b, p)
                    seen[p] = b
                    done[p[0]] = b + 1
    assert len(seen) == NH * (Sk // SR) and sorted(done) == list(range(NH))
    return bursts, [done[h] for h in range(NH)], J


def make(KB=256, NS=16, semchk=False, n4=16, n2=6, n1=4, vlead=1, lead=1, lead2=0.5, c_model=0.865,
         defer_norm=True, scoped=False, n_mid=128, flags=None, g_out=None,
         dB=(2, 2, 2, 2, 2, 2, 2, 2), dD=(2, 2, 2, 2, 2, 2, 2, 2), st_at=-1, pin=0, wr_rows=144, vgap=(), epi=True, e_first=False, wr_at=0, n_early=0, wr_alt=False, pin_mid=None, pin_epi=None):
    pin_mid = pin if pin_mid is None else pin_mid
    pin_epi = pin if pin_epi is None else pin_epi
    def f(x, k_cache, v_cache, wq, wo):
        B, Sq, D = x.shape
        _, H, Sk, Dh = k_cache.shape
        NH = B * H
        nkb = Sk // KB
        qscale = (Dh ** -0.5) * math.log2(math.e)
        k3 = k_cache.reshape(NH, Sk, Dh)
        v3 = v_cache.reshape(NH, Sk, Dh)
        x2 = x.reshape(B * Sq, D)
        wot = wo.T
        bursts, done, J = build_bursts(NH, Sk, n4, n2, n1)
        NB = len(bursts)
        n_pair_heads = 2 * J
        need = [0] * (NH + 1)
        for g in reversed(range(NH)):
            need[g] = max(done[g] + lead, need[g + 1] - 2)
        nus = [need[0]]; skips = []
        now = done[0]
        for g in range(NH):
            now = max(now + 2 * c_model, done[min(g + 1, NH - 1)])
            if nus[-1] + 1 >= max(need[g + 1], now + lead2):
                skips.append(g); nus.append(nus[-1] + 1)
            else:
                nus.append(nus[-1] + 2)
            assert nus[g] >= done[g], (g, nus[g], done[g])
            for b in range(nus[g], min(nus[g + 1] + vlead, NB)):
                for d in bursts[b][1]:
                    assert d is None or d[1] + (d[0] == PAIR) - NS < g
        assert nus[NH] >= NB
        last_issue = max(g for g in range(NH) if nus[g] < NB)
        skips = [g for g in skips if g <= last_issue]
        go = g_out if g_out is not None else last_issue
        assert go > NH - H
        def word(step, d):
            return 0 if d is None else (d[0] << 28) | ((step // SR) << 20) | (d[1] << 11) | d[2]
        words = [[word(step, d) for d in lanes] for step, lanes in bursts]
        NT_ = nus[NH] + vlead + 1
        words += [[0] * LANES] * (NT_ - NB)
        regular = lambda b, i: (PAIR << 28) | (1 << 20) | (((b >> 2) - 3 + i) << 12) | ((b & 15) << 7)
        b_lo = 12
        b_hi = next(b for b in range(b_lo, NB) if words[b] != [regular(b, i) for i in range(LANES)])
        gaps = [NB - gp + i for i, gp in enumerate(sorted(vgap, reverse=True))]
        f.info = dict(NB=NB, last_issue=last_issue, skips=skips, b_hi=b_hi, ahead=[nus[g] - done[g] for g in range(n_pair_heads - 8, NH)])

        def kern(x_hbm, k_hbm, v_hbm, wq_hbm, wo_hbm, out_hbm,
                 xb, wqb, wob, kvb, sb, qb, ob, lb, acc, outb, tab, semkv, semw, semo):
            def start_desc(tt, kind, w, k):
                src = (k_hbm, v_hbm)[tt]
                dst = kvb.at[tt]
                h = lax.shift_right_logical(w, 11) & (NH - 1)
                s = h & (NS - 1)
                row = (w & (Sk - 1)) + k * SR * (lax.shift_right_logical(w, 20) & 7)
                rows = pl.ds(pl.multiple_of(row, SR), SR)
                if kind == PAIR:
                    c = pltpu.make_async_copy(src.at[pl.ds(h, 2), rows], dst.at[pl.ds(s, 2), rows], semkv.at[tt, s])
                else:
                    c = pltpu.make_async_copy(src.reshape(2 * NH, Sk // 2, Dh).at[pl.ds(2 * h, 2), rows],
                                              dst.reshape(2 * NS, Sk // 2, Dh).at[pl.ds(2 * s, 2), rows], semkv.at[tt, s])
                c.start(priority=tt)
            def wait_item(tt, g):
                s = g & (NS - 1)
                @pl.when(jnp.logical_and(g < n_pair_heads, (g & 1) == 0))
                def _():
                    d = kvb.at[tt, pl.ds(s, 2)]
                    pltpu.make_async_copy(d, d, semkv.at[tt, s]).wait()
                @pl.when(g >= n_pair_heads)
                def _():
                    d = kvb.at[tt, s]
                    pltpu.make_async_copy(d, d, semkv.at[tt, s]).wait()

            nrt = D // 8
            def wloop(j, _):
                rt = lax.rem(j, 7) * 4 + lax.div(j, 7)
                for quarter in range(4):
                    for prio, (src, dst, si) in enumerate(((wq_hbm, wqb, 0), (wo_hbm, wob, 1))):
                        idx = (slice(None), pl.ds(pl.multiple_of(rt * 8, 8), 8), pl.ds(quarter * 1024, 1024))
                        pltpu.make_async_copy(src.reshape(2, D // 2, H * Dh).at[idx], dst.reshape(2, D // 2, H * Dh).at[idx],
                                              semw.at[si]).start(priority=prio)
                return 0
            lax.fori_loop(0, nrt // 2, wloop, 0)
            def tloop(b, _):
                for i in range(LANES):
                    tab[LANES * b + i] = jnp.where((b >> 2) + i >= 3, regular(b, i), 0)
                return 0
            lax.fori_loop(0, b_hi, tloop, 0)
            def xloop(j, _):
                for half in range(2):
                    idx = (slice(None), pl.ds(pl.multiple_of(j * 16 + half * (B * Sq // 4), 16), 16))
                    pltpu.make_async_copy(x_hbm.reshape(2, B * Sq // 2, D).at[idx], xb.reshape(2, B * Sq // 2, D).at[idx],
                                          semw.at[2]).start(priority=half)
                return 0
            lax.fori_loop(0, B * Sq // 64, xloop, 0)
            def kvloop(i, _):
                for k in range(DEPTH):
                    for ln in range(LANES):
                        for tt in range(2):
                            w = tab[LANES * (i if tt else jnp.maximum(i - vlead, 0)) + ln]
                            ok = w != 0
                            if not tt:
                                ok = jnp.logical_and(ok, i >= vlead)
                            pl.when(ok)(functools.partial(start_desc, tt, PAIR, w, k))
                return 0
            assert nus[0] + vlead <= b_hi
            lax.fori_loop(0, nus[0] + vlead, kvloop, 0)
            for b in range(b_hi, NT_):
                for i in range(LANES):
                    tab[LANES * b + i] = jnp.int32(words[b][i])
            for dst, si in ((wqb, 0), (wob, 1), (xb, 2)):
                pltpu.make_async_copy(dst, dst, semw.at[si]).wait()

            def qproj(g):
                b = g // H if isinstance(g, int) else lax.shift_right_logical(g, 4)
                h = g % H if isinstance(g, int) else g & (H - 1)
                w = wqb[:, pl.ds(pl.multiple_of(h * Dh, Dh), Dh)]
                xx = xb[pl.ds(pl.multiple_of(b * Sq, 16), Sq), :]
                q = jnp.dot(xx, w, preferred_element_type=jnp.float32)
                return (q * qscale).astype(jnp.bfloat16)

            def outproj(g):
                h = g % H if isinstance(g, int) else g & (H - 1)
                w = wob[:, pl.ds(pl.multiple_of(h * Dh, Dh), Dh)]
                if defer_norm:
                    l = jnp.sum(lb[...], axis=-1, keepdims=True)
                    o = (ob[...] * (1.0 / l)).astype(jnp.bfloat16)
                else:
                    o = ob[...]
                return lax.dot_general(o, w, NT, preferred_element_type=jnp.float32)

            sc = lambda n: jax.named_scope(n) if scoped else contextlib.nullcontext()

            def scores(s, dma):
                q = qb[...]
                m = None
                for t in range(nkb):
                    kt = kvb[0, s, pl.ds(t * KB, KB), :]
                    dma(t)
                    st = lax.dot_general(q, kt, NT, preferred_element_type=jnp.float32)
                    sb[:, pl.ds(t * KB, KB)] = st
                    for u in range(KB // 128):
                        su = st[:, u * 128:(u + 1) * 128]
                        m = su if m is None else jnp.maximum(m, su)
                return jnp.max(m, axis=-1, keepdims=True)

            def values(s, m, dma, zero, pin):
                o = None; l = None
                pend = []
                ocols = pl.ds(pl.multiple_of(Sk + zero, Dh), Dh) if pin else None
                for t in range(nkb):
                    vt = kvb[1, s, pl.ds(t * KB, KB), :]
                    dma(nkb + t)
                    if pin and len(pend) >= pin:
                        ot = pend.pop(0)
                        sb[:, ocols] = ot if t == pin else sb[:, ocols] + ot
                    p = jnp.exp2(sb[:, pl.ds(t * KB, KB)] - m)
                    for u in range(KB // 128):
                        pu = p[:, u * 128:(u + 1) * 128]
                        l = pu if l is None else l + pu
                    ot = jnp.dot(p.astype(jnp.bfloat16), vt, preferred_element_type=jnp.float32)
                    if pin:
                        pend.append(ot)
                    else:
                        o = ot if o is None else o + ot
                if pin:
                    o = sb[:, ocols]
                    for ot in pend:
                        o = o + ot
                return o, l

            def body(g, b0, midwait):
                s = g & (NS - 1)
                zero = lax.shift_right_logical(g, 20) * Dh
                second = functools.reduce(jnp.logical_and, [g != sk for sk in skips], g >= 0)
                par = {}
                cuts = [0]
                for c_ in tuple(dB) + tuple(dD):
                    cuts.append(cuts[-1] + c_)
                assert cuts[-1] == 2 * LANES * DEPTH and len(cuts) == 2 * nkb + 1
                def dma(blk):
                    for i in range(cuts[blk], cuts[blk + 1]):
                        half, k, ln = i // (LANES * DEPTH), (i // LANES) % DEPTH, i % LANES
                        for tt in range(2):
                            key = (half, tt, ln)
                            if key not in par:
                                if tt == 0:
                                    w = tab[LANES * b0 + (LANES * half + ln)]
                                else:
                                    slot = b0 + (half + vlead)
                                    bv = slot
                                    for gp in gaps:
                                        bv = bv - (slot > gp).astype(jnp.int32)
                                    w = tab[LANES * bv + ln]
                                    for gp in gaps:
                                        w = jnp.where(slot == gp, 0, w)
                                if half:
                                    w = jnp.where(second, w, 0)
                                par[key] = w
                            w = par[key]
                            for kind in (PAIR, SINGLE):
                                pl.when(lax.shift_right_logical(w, 28) == kind)(functools.partial(start_desc, tt, kind, w, k))
                with sc("wk"):
                    wait_item(0, g)
                if not midwait:
                    with sc("wv"):
                        wait_item(1, g)
                m = scores(s, dma)
                qn = qproj(jnp.minimum(g + 1, NH - 1))
                y = outproj(g - 1)
                qb[...] = qn
                fresh = ((g - 1) & (H - 1)) == 0
                acc[...] = jnp.where(fresh, y, acc[...] + y)
                if midwait:
                    with sc("wv"):
                        wait_item(1, g)
                o, l = values(s, m, dma, zero, pin_mid if midwait else pin)
                if defer_norm:
                    ob[...] = o
                    lb[...] = l
                else:
                    l = jnp.sum(l, axis=-1, keepdims=True)
                    ob[...] = (o * (1.0 / l)).astype(jnp.bfloat16)

                @pl.when(jnp.logical_and((g & (H - 1)) == 0, g > 0))
                def _():
                    b = lax.shift_right_logical(jnp.maximum(g - 1, 0), 4)
                    outb[pl.ds(pl.multiple_of(b * Sq, 16), Sq), :] = acc[...].astype(jnp.bfloat16)
                if n_early:
                    pl.when(g == n_early * H + 1)(functools.partial(write_out, 0, n_early))
                return b0 + 1 + second.astype(jnp.int32)

            def write_out(b0, b1):
                n = (b1 - b0) * Sq // wr_rows
                assert n * wr_rows == (b1 - b0) * Sq and wr_rows % 8 == 0
                for j in range(n):
                    jj = j // 2 + (j % 2) * ((n + 1) // 2)
                    r = pl.ds(b0 * Sq + jj * wr_rows, wr_rows)
                    pltpu.make_async_copy(outb.at[r], out_hbm.at[r], semo.at[0]).start(priority=j % 2 if wr_alt else 0)

            qb[...] = qproj(0)
            acc[...] = jnp.zeros_like(acc)
            ob[...] = jnp.zeros_like(ob)
            lb[...] = jnp.ones_like(lb)
            def sbody(g, c, midwait):
                with sc("it"):
                    return body(g, c, midwait)
            bb = nus[0]
            end = NH - 1 if epi else NH
            split = max(end - n_mid, 0)
            if split > 0:
                bb = lax.fori_loop(0, split, functools.partial(sbody, midwait=False), bb)
            if split < end:
                bb = lax.fori_loop(split, end, functools.partial(sbody, midwait=True), bb)
            last = pl.ds((B - 1) * Sq, Sq)
            if epi:
                assert last_issue < NH - 1
                g = NH - 1
                s = g & (NS - 1)
                with sc("it"):
                    if e_first:
                        acc[...] += outproj(g - 1)
                    with sc("wk"):
                        d = kvb.at[0, s]
                        pltpu.make_async_copy(d, d, semkv.at[0, s]).wait()
                    m = scores(s, lambda blk: write_out(n_early, B - 1) if blk == wr_at else None)
                    if not e_first:
                        acc[...] += outproj(g - 1)
                    with sc("wv"):
                        d = kvb.at[1, s]
                        pltpu.make_async_copy(d, d, semkv.at[1, s]).wait()
                    if wr_at >= nkb:
                        write_out(n_early, B - 1)
                    o, l = values(s, m, lambda blk: None, lax.shift_right_logical(bb, 20) * Dh, pin_epi)
                    l = jnp.sum(l, axis=-1, keepdims=True)
                    o = (o * (1.0 / l)).astype(jnp.bfloat16)
                    y = lax.dot_general(o, wob[:, pl.ds((H - 1) * Dh, Dh)], NT, preferred_element_type=jnp.float32)
                    outb[last, :] = (acc[...] + y).astype(jnp.bfloat16)
            else:
                outb[last, :] = (acc[...] + outproj(NH - 1)).astype(jnp.bfloat16)
            co = pltpu.make_async_copy(outb.at[last], out_hbm.at[last], semo.at[1])
            co.start()
            rest = outb.at[pl.ds(0, (B - 1) * Sq)]
            with sc("wo1"):
                pltpu.make_async_copy(rest, rest, semo.at[0]).wait()
            with sc("wo2"):
                co.wait()

        hbm = pl.BlockSpec(memory_space=pltpu.HBM)
        out = pl.pallas_call(
            kern,
            in_specs=[hbm] * 5,
            out_specs=hbm,
            out_shape=jax.ShapeDtypeStruct((B * Sq, D), x.dtype),
            scratch_shapes=[
                pltpu.VMEM((B * Sq, D), jnp.bfloat16),
                pltpu.VMEM((D, H * Dh), jnp.bfloat16),
                pltpu.VMEM((D, H * Dh), jnp.bfloat16),
                pltpu.VMEM((2, NS, Sk, Dh), jnp.bfloat16),
                pltpu.VMEM((Sq, Sk + (2 * Dh if pin or pin_mid or pin_epi else 0)), jnp.float32),
                pltpu.VMEM((Sq, Dh), jnp.bfloat16),
                pltpu.VMEM((Sq, Dh), jnp.float32 if defer_norm else jnp.bfloat16),
                pltpu.VMEM((Sq, 128), jnp.float32),
                pltpu.VMEM((Sq, D), jnp.float32),
                pltpu.VMEM((B * Sq, D), jnp.bfloat16),
                pltpu.SMEM((NT_ * LANES,), jnp.int32),
                pltpu.SemaphoreType.DMA((2, NS)),
                pltpu.SemaphoreType.DMA((3,)),
                pltpu.SemaphoreType.DMA((2,)),
            ],
            compiler_params=pltpu.CompilerParams(vmem_limit_bytes=100 * 1024 * 1024, disable_bounds_checks=True,
                                                 disable_semaphore_checks=not semchk, flags=flags),
        )(x2, k3, v3, wq, wot)
        return out.reshape(B, Sq, D)
    return f


@jax.jit
def pallas_standalone__mha_block_cached__near_ridge_kernel(x, k_cache, v_cache, wq, wo):
    return make(pin=2,pin_mid=2,c_model=0.85,n_mid=128,lead=1,lead2=1,vlead=1,n4=20,n2=12,n1=6,wr_at=8)(x, k_cache, v_cache, wq, wo)
```

```python
import functools
import math

import jax
import jax.numpy as jnp
from jax import lax
import jax.experimental.pallas as pl
import jax.experimental.pallas.tpu as pltpu

_SEG = 32
_LANES = 4
_DEPTH = 4
_BURST = _LANES * _DEPTH
_SLOTS = 16
_KB = 256
_V_BACK = 4
_TAPER = (20, 12, 6)
_EMPTY, _PAIR, _SINGLE = 0, 1, 2
_KIND_SHIFT, _STEP_SHIFT = 28, 24
_NT_DIMS = (((1,), (1,)), ((), ()))


def _plan_bursts(n_heads, sk):
    n4, n2, n1 = _TAPER
    life = sk // _SEG
    period = life // _LANES
    n_pairs = (n_heads - n4 - n2 - n1) // 2
    assert n_pairs >= _LANES and 2 * n_pairs + n4 + n2 + n1 == n_heads and n4 % 2 == 0
    end4 = n_pairs + n4 // 2
    end2 = end4 + n2
    end1 = end2 + 2 * n1

    def lane(t, a):
        j = t // period - (_LANES - 1) + a
        if j < 0:
            return None
        if j < n_pairs:
            return _PAIR, 2 * j, t % life * _SEG
        row = t % (life // 2) * _SEG
        if a < _LANES // 2:
            return (_SINGLE, 2 * j + 2, row) if j < end4 else None
        if j >= end1 or (j >= end2 and (j - end2) % 2):
            return None
        return _SINGLE, min(max(j + n_pairs, 2 * j - 1), j + end4, (j + end2) // 2 + end4), row

    bursts = []
    t = 0
    while t < period * end1:
        lanes = [lane(t, a) for a in range(_LANES)]
        active = [d for d in lanes if d is not None]
        if len(active) > _LANES // 2 or t < life:
            bursts.append((_SEG, lanes))
            t += _DEPTH
        else:
            rep = _LANES // len(active)
            bursts.append((rep * _SEG, [(k, h, r + i * _SEG) for i in range(rep) for k, h, r in active]))
            t += rep * _DEPTH

    seen = {}
    done = [0] * n_heads
    for b, (step, lanes) in enumerate(bursts):
        for kind, h, row in (d for d in lanes if d is not None):
            for r in range(row, row + _DEPTH * step, step):
                assert r + _SEG <= (sk if kind == _PAIR else sk // 2)
                for part in ((h, r), (h + 1, r) if kind == _PAIR else (h, r + sk // 2)):
                    assert part not in seen
                    seen[part] = b
                    done[part[0]] = b + 1
    assert len(seen) == n_heads * life
    return bursts, done, 2 * n_pairs


def _plan_issue(bursts, done, compute_cost=0.85, lead=1):
    n_heads = len(done)
    need = [0] * (n_heads + 1)
    for g in reversed(range(n_heads)):
        need[g] = max(done[g] + lead, need[g + 1] - 2)
    issued, skips = [need[0]], []
    now = done[0]
    for g in range(n_heads - 1):
        now = max(now + 2 * compute_cost, done[g + 1])
        skip = issued[-1] + 1 >= max(need[g + 1], now + lead) and issued[-1] < len(bursts)
        if skip:
            skips.append(g)
        issued.append(issued[-1] + (1 if skip else 2))
    assert issued[-1] >= len(bursts)
    for g in range(n_heads - 1):
        assert issued[g] >= done[g]
        for _, lanes in bursts[issued[g]:issued[g + 1] + 1]:
            assert all(d is None or d[1] + (d[0] == _PAIR) - _SLOTS < g for d in lanes)
    return issued, skips


def _kernel(x_hbm, k_hbm, v_hbm, wq_hbm, wo_hbm, out_hbm,
            x_buf, wq_buf, wo_buf, kv_buf, s_buf, q_buf, o_buf, l_buf, acc, out_buf,
            table, kv_sem, in_sem, out_sem, *, batch, heads):
    n_heads, sk, dh = k_hbm.shape
    d_model = wq_hbm.shape[0]
    sq = x_hbm.shape[0] // batch
    n_kb = sk // _KB
    row_bits = sk.bit_length() - 1
    head_bits = heads.bit_length() - 1
    assert sk == 1 << row_bits and heads == 1 << head_bits
    q_scale = dh ** -0.5 * math.log2(math.e)

    bursts, done, paired_heads = _plan_bursts(n_heads, sk)
    issued, skips = _plan_issue(bursts, done)

    def encode(step, d):
        if d is None:
            return _EMPTY
        return d[0] << _KIND_SHIFT | step // _SEG << _STEP_SHIFT | d[1] << row_bits | d[2]

    def steady_word(b, a):
        per = sk // _SEG // _LANES // _DEPTH
        pair = lax.div(b, per) + (a - (_LANES - 1))
        row = lax.rem(b, _LANES * per) * (_DEPTH * _SEG)
        word = (_PAIR << _KIND_SHIFT | 1 << _STEP_SHIFT) + pair * (2 * sk) + row
        return jnp.where(pair >= 0, word, _EMPTY)

    words = [[encode(step, d) for d in lanes] for step, lanes in bursts]
    words += [[_EMPTY] * _LANES] * (table.shape[0] // _LANES - len(words))
    n_steady = next(b for b, (_, lanes) in enumerate(bursts) if any(d and d[0] == _SINGLE for d in lanes))

    def start_load(cache, kind, word, depth):
        src = (k_hbm, v_hbm)[cache]
        dst = kv_buf.at[cache]
        head = lax.shift_right_logical(word & ((1 << _STEP_SHIFT) - 1), row_bits)
        slot = head & (_SLOTS - 1)
        step = lax.shift_right_logical(word, _STEP_SHIFT) & ((1 << _KIND_SHIFT - _STEP_SHIFT) - 1)
        rows = pl.ds(pl.multiple_of((word & (sk - 1)) + depth * _SEG * step, _SEG), _SEG)
        if kind == _PAIR:
            src = src.at[pl.ds(head, 2), rows]
            dst = dst.at[pl.ds(slot, 2), rows]
        else:
            src = src.reshape(2 * n_heads, sk // 2, dh).at[pl.ds(2 * head, 2), rows]
            dst = dst.reshape(2 * _SLOTS, sk // 2, dh).at[pl.ds(2 * slot, 2), rows]
        pltpu.make_async_copy(src, dst, kv_sem.at[cache, slot]).start(priority=cache)

    def wait_all(buf, sem):
        pltpu.make_async_copy(buf, buf, sem).wait()

    def wait_head(cache, g):
        slot = g & (_SLOTS - 1)

        @pl.when(jnp.logical_and(g < paired_heads, (g & 1) == 0))
        def _():
            wait_all(kv_buf.at[cache, pl.ds(slot, 2)], kv_sem.at[cache, slot])

        @pl.when(g >= paired_heads)
        def _():
            wait_all(kv_buf.at[cache, slot], kv_sem.at[cache, slot])

    x_rows = 32
    n_x = batch * sq // x_rows
    x_first = n_x // 4 * 2 - 2
    assert n_x * x_rows == batch * sq and n_x % 2 == 0

    def start_x(j, priority):
        rows = pl.ds(pl.multiple_of(j * x_rows, x_rows), x_rows)
        pltpu.make_async_copy(x_hbm.at[rows], x_buf.at[rows], in_sem.at[2]).start(priority=priority)

    w_cols = 1024
    w_tiles = d_model // 2 // _LANES // 8
    assert w_tiles * 2 * _LANES * 8 == d_model

    def start_weights(j, _):
        halves = (2, d_model // 2, heads * dh)
        for c in range(0, heads * dh, w_cols):
            for a in range(_LANES):
                idx = (slice(None), pl.ds(pl.multiple_of((j + a * w_tiles) * 8, 8), 8), pl.ds(c, w_cols))
                for i, (src, dst) in enumerate(((wq_hbm, wq_buf), (wo_hbm, wo_buf))):
                    pltpu.make_async_copy(src.reshape(*halves).at[idx], dst.reshape(*halves).at[idx],
                                          in_sem.at[i]).start(priority=i)
        return 0

    def fill_table(b, _):
        for a in range(_LANES):
            table[_LANES * b + a] = steady_word(b, a)
        return 0

    def start_x_rest(j, _):
        for half in range(2):
            start_x(x_first + j + half * ((n_x - x_first) // 2), half)
        return 0

    def start_first_bursts(b, _):
        for depth in range(_DEPTH):
            for a in range(_LANES):
                for cache in range(2):
                    word = table[_LANES * (b if cache else jnp.maximum(b - 1, 0)) + a]
                    live = word != _EMPTY
                    if cache == 0:
                        live = jnp.logical_and(live, b >= 1)
                    elif depth * _LANES >= _BURST - _V_BACK:
                        live = jnp.logical_and(live, b < issued[0])
                    pl.when(live)(functools.partial(start_load, cache, _PAIR, word, depth))
        return 0

    for j in range(x_first):
        start_x(j, 1)
    lax.fori_loop(0, w_tiles, start_weights, 0)
    lax.fori_loop(0, n_steady, fill_table, 0)
    lax.fori_loop(0, (n_x - x_first) // 2, start_x_rest, 0)
    assert issued[0] + 1 <= n_steady
    lax.fori_loop(0, issued[0] + 1, start_first_bursts, 0)
    for b in range(n_steady, len(words)):
        for a in range(_LANES):
            table[_LANES * b + a] = jnp.int32(words[b][a])
    for i, buf in enumerate((wq_buf, wo_buf, x_buf)):
        wait_all(buf, in_sem.at[i])

    def head_cols(g):
        h = g & (heads - 1)
        return pl.ds(h * dh if isinstance(h, int) else pl.multiple_of(h * dh, dh), dh)

    def batch_rows(b):
        return pl.ds(b * sq if isinstance(b, int) else pl.multiple_of(b * sq, 16), sq)

    def project_q(g):
        b = g >> head_bits if isinstance(g, int) else lax.shift_right_logical(g, head_bits)
        q = jnp.dot(x_buf[batch_rows(b), :], wq_buf[:, head_cols(g)], preferred_element_type=jnp.float32)
        return (q * q_scale).astype(q_buf.dtype)

    def project_out(g, o, l):
        o = (o * (1.0 / jnp.sum(l, axis=-1, keepdims=True))).astype(wo_buf.dtype)
        return lax.dot_general(o, wo_buf[:, head_cols(g)], _NT_DIMS, preferred_element_type=jnp.float32)

    def lane_tiles(a):
        return [a[:, i:i + 128] for i in range(0, a.shape[1], 128)]

    def scores(slot, between):
        q = q_buf[...]
        tiles = []
        for t in range(n_kb):
            keys = pl.ds(t * _KB, _KB)
            k = kv_buf[0, slot, keys, :]
            between(t)
            s = lax.dot_general(q, k, _NT_DIMS, preferred_element_type=jnp.float32)
            s_buf[:, keys] = s
            tiles += lane_tiles(s)
        return jnp.max(functools.reduce(jnp.maximum, tiles), axis=-1, keepdims=True)

    def weighted_values(slot, m, between, zero):
        total = pl.ds(pl.multiple_of(sk + zero, dh), dh)
        pending, tiles = [], []
        for t in range(n_kb):
            keys = pl.ds(t * _KB, _KB)
            v = kv_buf[1, slot, keys, :]
            between(n_kb + t)
            if len(pending) == 2:
                part = pending.pop(0)
                s_buf[:, total] = part if t == 2 else s_buf[:, total] + part
            p = jnp.exp2(s_buf[:, keys] - m)
            tiles += lane_tiles(p)
            pending.append(jnp.dot(p.astype(v.dtype), v, preferred_element_type=jnp.float32))
        return functools.reduce(jnp.add, pending, s_buf[:, total]), functools.reduce(jnp.add, tiles)

    def head_step(g, burst):
        slot = g & (_SLOTS - 1)
        second = functools.reduce(jnp.logical_and, [g != s for s in skips], g >= 0)
        lane_words = {}

        def issue(block):
            per_block = _BURST // n_kb
            for i in range(block * per_block, (block + 1) * per_block):
                for cache in range(2):
                    n = i + cache * (_BURST - _V_BACK)
                    key = (n // _BURST, n % _LANES, i >= _BURST)
                    if key not in lane_words:
                        word = table[_LANES * burst + (_LANES * key[0] + key[1])]
                        lane_words[key] = jnp.where(second, word, _EMPTY) if key[2] else word
                    word = lane_words[key]
                    for kind in (_PAIR, _SINGLE):
                        pl.when(lax.shift_right_logical(word, _KIND_SHIFT) == kind)(
                            functools.partial(start_load, cache, kind, word, n // _LANES % _DEPTH))

        wait_head(0, g)
        m = scores(slot, issue)
        q_next = project_q(g + 1)
        y = project_out(g - 1, o_buf[...], l_buf[...])
        q_buf[...] = q_next
        acc[...] = jnp.where(((g - 1) & (heads - 1)) == 0, y, acc[...] + y)
        wait_head(1, g)
        o_buf[...], l_buf[...] = weighted_values(slot, m, issue, lax.shift_right_logical(g, 20) * dh)

        @pl.when(jnp.logical_and((g & (heads - 1)) == 0, g > 0))
        def _():
            b = lax.shift_right_logical(jnp.maximum(g - 1, 0), head_bits)
            out_buf[batch_rows(b), :] = acc[...].astype(out_buf.dtype)

        return burst + 1 + second.astype(jnp.int32)

    q_buf[...] = project_q(0)
    acc[...] = jnp.zeros_like(acc)
    o_buf[...] = jnp.zeros_like(o_buf)
    l_buf[...] = jnp.ones_like(l_buf)
    burst = lax.fori_loop(0, n_heads - 1, head_step, issued[0])

    def store(b, sem):
        return pltpu.make_async_copy(out_buf.at[batch_rows(b)], out_hbm.at[batch_rows(b)], sem)

    g = n_heads - 1
    slot = g & (_SLOTS - 1)
    wait_all(kv_buf.at[0, slot], kv_sem.at[0, slot])
    m = scores(slot, lambda block: None)
    wait_all(kv_buf.at[1, slot], kv_sem.at[1, slot])
    for b in range(batch - 1):
        store(b, out_sem.at[0]).start()
    acc[...] += project_out(g - 1, o_buf[...], l_buf[...])
    o, l = weighted_values(slot, m, lambda block: None, lax.shift_right_logical(burst, 20) * dh)
    out_buf[batch_rows(batch - 1), :] = (acc[...] + project_out(g, o, l)).astype(out_buf.dtype)
    last = store(batch - 1, out_sem.at[1])
    last.start()
    wait_all(out_buf.at[pl.ds(0, (batch - 1) * sq)], out_sem.at[0])
    last.wait()


@jax.jit
def pallas_standalone__mha_block_cached__near_ridge_kernel(
    x: jax.Array,
    k_cache: jax.Array,
    v_cache: jax.Array,
    wq: jax.Array,
    wo: jax.Array,
):
    batch, sq, d_model = x.shape
    _, heads, sk, dh = k_cache.shape
    bursts, done, _ = _plan_bursts(batch * heads, sk)
    issued, _ = _plan_issue(bursts, done)

    hbm = pl.BlockSpec(memory_space=pltpu.HBM)
    out = pl.pallas_call(
        functools.partial(_kernel, batch=batch, heads=heads),
        in_specs=[hbm] * 5,
        out_specs=hbm,
        out_shape=jax.ShapeDtypeStruct((batch * sq, d_model), x.dtype),
        scratch_shapes=[
            pltpu.VMEM((batch * sq, d_model), x.dtype),
            pltpu.VMEM((d_model, heads * dh), wq.dtype),
            pltpu.VMEM((d_model, heads * dh), wo.dtype),
            pltpu.VMEM((2, _SLOTS, sk, dh), k_cache.dtype),
            pltpu.VMEM((sq, sk + 2 * dh), jnp.float32),
            pltpu.VMEM((sq, dh), x.dtype),
            pltpu.VMEM((sq, dh), jnp.float32),
            pltpu.VMEM((sq, 128), jnp.float32),
            pltpu.VMEM((sq, d_model), jnp.float32),
            pltpu.VMEM((batch * sq, d_model), x.dtype),
            pltpu.SMEM(((issued[-1] + 2) * _LANES,), jnp.int32),
            pltpu.SemaphoreType.DMA((2, _SLOTS)),
            pltpu.SemaphoreType.DMA((3,)),
            pltpu.SemaphoreType.DMA((2,)),
        ],
        compiler_params=pltpu.CompilerParams(
            vmem_limit_bytes=100 * 1024 * 1024,
            disable_bounds_checks=True,
            disable_semaphore_checks=True,
        ),
    )(
        x.reshape(batch * sq, d_model),
        k_cache.reshape(batch * heads, sk, dh),
        v_cache.reshape(batch * heads, sk, dh),
        wq,
        wo.T,
    )
    return out.reshape(batch, sq, d_model)
```

```python
import functools
import math

import jax
import jax.numpy as jnp
from jax import lax
import jax.experimental.pallas as pl
import jax.experimental.pallas.tpu as pltpu

_SEG = 32
_LANES = 4
_DEPTH = 4
_BURST = _LANES * _DEPTH
_SLOTS = 16
_KB = 256
_V_BACK = 4
_TAPER = (20, 12, 6)
_EMPTY, _PAIR, _SINGLE = 0, 1, 2
_KIND_SHIFT, _STEP_SHIFT = 28, 24
_NT_DIMS = (((1,), (1,)), ((), ()))


def _plan_bursts(n_heads, sk):
    n4, n2, n1 = _TAPER
    life = sk // _SEG
    period = life // _LANES
    n_pairs = (n_heads - n4 - n2 - n1) // 2
    assert n_pairs >= _LANES and 2 * n_pairs + n4 + n2 + n1 == n_heads and n4 % 2 == 0
    end4 = n_pairs + n4 // 2
    end2 = end4 + n2
    end1 = end2 + 2 * n1

    def lane(t, a):
        j = t // period - (_LANES - 1) + a
        if j < 0:
            return None
        if j < n_pairs:
            return _PAIR, 2 * j, t % life * _SEG
        row = t % (life // 2) * _SEG
        if a < _LANES // 2:
            return (_SINGLE, 2 * j + 2, row) if j < end4 else None
        if j >= end1 or (j >= end2 and (j - end2) % 2):
            return None
        return _SINGLE, min(max(j + n_pairs, 2 * j - 1), j + end4, (j + end2) // 2 + end4), row

    bursts = []
    t = 0
    while t < period * end1:
        lanes = [lane(t, a) for a in range(_LANES)]
        active = [d for d in lanes if d is not None]
        if len(active) > _LANES // 2 or t < life:
            bursts.append((_SEG, lanes))
            t += _DEPTH
        else:
            rep = _LANES // len(active)
            bursts.append((rep * _SEG, [(k, h, r + i * _SEG) for i in range(rep) for k, h, r in active]))
            t += rep * _DEPTH

    seen = {}
    done = [0] * n_heads
    for b, (step, lanes) in enumerate(bursts):
        for kind, h, row in (d for d in lanes if d is not None):
            for r in range(row, row + _DEPTH * step, step):
                assert r // (sk // 2) == row // (sk // 2) and (kind == _PAIR or r < sk // 2)
                for part in ((h, r), (h + 1, r) if kind == _PAIR else (h, r + sk // 2)):
                    assert part not in seen
                    seen[part] = b
                    done[part[0]] = b + 1
    assert len(seen) == n_heads * life
    return bursts, done, 2 * n_pairs


def _plan_issue(bursts, done, compute_cost=0.85, lead=1):
    n_heads = len(done)
    need = [0] * (n_heads + 1)
    for g in reversed(range(n_heads)):
        need[g] = max(done[g] + lead, need[g + 1] - 2)
    issued, skips = [need[0]], []
    now = done[0]
    for g in range(n_heads - 1):
        now = max(now + 2 * compute_cost, done[g + 1])
        skip = issued[-1] + 1 >= max(need[g + 1], now + lead) and issued[-1] < len(bursts)
        if skip:
            skips.append(g)
        issued.append(issued[-1] + (1 if skip else 2))
    assert issued[-1] >= len(bursts)
    for g in range(n_heads - 1):
        assert issued[g] >= done[g]
        for _, lanes in bursts[issued[g]:issued[g + 1] + 1]:
            assert all(d is None or d[1] + (d[0] == _PAIR) - _SLOTS < g for d in lanes)
    return issued, skips


def _kernel(x_hbm, k_hbm, v_hbm, wq_hbm, wo_hbm, out_hbm,
            x_buf, wq_buf, wo_buf, kv_buf, s_buf, q_buf, o_buf, l_buf, acc, out_buf,
            table, kv_sem, in_sem, out_sem, *, batch, heads):
    n_heads, _, half_sk, dh = k_hbm.shape
    sk = 2 * half_sk
    half_d = wq_hbm.shape[1]
    sq = x_hbm.shape[0] // batch
    n_kb = sk // _KB
    row_bits = sk.bit_length() - 1
    head_bits = heads.bit_length() - 1
    assert sk == 1 << row_bits and heads == 1 << head_bits
    q_scale = dh ** -0.5 * math.log2(math.e)

    bursts, done, paired_heads = _plan_bursts(n_heads, sk)
    issued, skips = _plan_issue(bursts, done)

    def encode(step, d):
        if d is None:
            return _EMPTY
        return d[0] << _KIND_SHIFT | step // _SEG << _STEP_SHIFT | d[1] << row_bits | d[2]

    def steady_word(b, a):
        per = sk // _SEG // _LANES // _DEPTH
        pair = lax.div(b, per) + (a - (_LANES - 1))
        row = lax.rem(b, _LANES * per) * (_DEPTH * _SEG)
        word = (_PAIR << _KIND_SHIFT | 1 << _STEP_SHIFT) + pair * (2 * sk) + row
        return jnp.where(pair >= 0, word, _EMPTY)

    words = [[encode(step, d) for d in lanes] for step, lanes in bursts]
    words += [[_EMPTY] * _LANES] * (table.shape[0] // _LANES - len(words))
    n_steady = next(b for b, (_, lanes) in enumerate(bursts) if any(d and d[0] == _SINGLE for d in lanes))

    def start_load(cache, kind, word, depth):
        head = lax.shift_right_logical(word & ((1 << _STEP_SHIFT) - 1), row_bits)
        slot = head & (_SLOTS - 1)
        step = lax.shift_right_logical(word, _STEP_SHIFT) & ((1 << _KIND_SHIFT - _STEP_SHIFT) - 1)
        rows = pl.ds(pl.multiple_of((word & (half_sk - 1)) + depth * _SEG * step, _SEG), _SEG)
        if kind == _PAIR:
            half = lax.shift_right_logical(word, row_bits - 1) & 1
            src = (k_hbm, v_hbm)[cache].at[pl.ds(head, 2), half, rows]
            dst = kv_buf.at[cache, pl.ds(slot, 2), half, rows]
        else:
            src = (k_hbm, v_hbm)[cache].at[head, :, rows]
            dst = kv_buf.at[cache, slot, :, rows]
        pltpu.make_async_copy(src, dst, kv_sem.at[cache, slot]).start(priority=cache)

    def wait_all(buf, sem):
        pltpu.make_async_copy(buf, buf, sem).wait()

    def wait_head(cache, g):
        slot = g & (_SLOTS - 1)

        @pl.when(jnp.logical_and(g < paired_heads, (g & 1) == 0))
        def _():
            wait_all(kv_buf.at[cache, pl.ds(slot, 2)], kv_sem.at[cache, slot])

        @pl.when(g >= paired_heads)
        def _():
            wait_all(kv_buf.at[cache, slot], kv_sem.at[cache, slot])

    x_rows = 32
    n_x = batch * sq // x_rows
    x_first = n_x // 4 * 2 - 2
    assert n_x * x_rows == batch * sq and n_x % 2 == 0

    def start_x(j, priority):
        rows = pl.ds(pl.multiple_of(j * x_rows, x_rows), x_rows)
        pltpu.make_async_copy(x_hbm.at[rows], x_buf.at[rows], in_sem.at[2]).start(priority=priority)

    w_cols = 1024
    w_tiles = half_d // _LANES // 8
    assert w_tiles * _LANES * 8 == half_d

    def start_weights(j, _):
        for c in range(0, heads * dh, w_cols):
            for a in range(_LANES):
                idx = (slice(None), pl.ds(pl.multiple_of((j + a * w_tiles) * 8, 8), 8), pl.ds(c, w_cols))
                for i, (src, dst) in enumerate(((wq_hbm, wq_buf), (wo_hbm, wo_buf))):
                    pltpu.make_async_copy(src.at[idx], dst.at[idx], in_sem.at[i]).start(priority=i)
        return 0

    def fill_table(b, _):
        for a in range(_LANES):
            table[_LANES * b + a] = steady_word(b, a)
        return 0

    def start_x_rest(j, _):
        for half in range(2):
            start_x(x_first + j + half * ((n_x - x_first) // 2), half)
        return 0

    def start_first_bursts(b, _):
        for depth in range(_DEPTH):
            for a in range(_LANES):
                for cache in range(2):
                    word = table[_LANES * (b if cache else jnp.maximum(b - 1, 0)) + a]
                    live = word != _EMPTY
                    if cache == 0:
                        live = jnp.logical_and(live, b >= 1)
                    elif depth * _LANES >= _BURST - _V_BACK:
                        live = jnp.logical_and(live, b < issued[0])
                    pl.when(live)(functools.partial(start_load, cache, _PAIR, word, depth))
        return 0

    for j in range(x_first):
        start_x(j, 1)
    lax.fori_loop(0, w_tiles, start_weights, 0)
    lax.fori_loop(0, n_steady, fill_table, 0)
    lax.fori_loop(0, (n_x - x_first) // 2, start_x_rest, 0)
    assert issued[0] + 1 <= n_steady
    lax.fori_loop(0, issued[0] + 1, start_first_bursts, 0)
    for b in range(n_steady, len(words)):
        for a in range(_LANES):
            table[_LANES * b + a] = jnp.int32(words[b][a])
    for i, buf in enumerate((wq_buf, wo_buf, x_buf)):
        wait_all(buf, in_sem.at[i])

    def head_weights(w_buf, g):
        h = g & (heads - 1)
        cols = pl.ds(h * dh if isinstance(h, int) else pl.multiple_of(h * dh, dh), dh)
        return w_buf[:, :, cols].reshape(2 * half_d, dh)

    def cache_block(cache, slot, t):
        return kv_buf[cache, slot, t * _KB // half_sk, pl.ds(t * _KB % half_sk, _KB), :]

    def batch_rows(b):
        return pl.ds(b * sq if isinstance(b, int) else pl.multiple_of(b * sq, 16), sq)

    def project_q(g):
        b = g >> head_bits if isinstance(g, int) else lax.shift_right_logical(g, head_bits)
        q = jnp.dot(x_buf[batch_rows(b), :], head_weights(wq_buf, g), preferred_element_type=jnp.float32)
        return (q * q_scale).astype(q_buf.dtype)

    def project_out(g, o, l):
        o = (o * (1.0 / jnp.sum(l, axis=-1, keepdims=True))).astype(wo_buf.dtype)
        return lax.dot_general(o, head_weights(wo_buf, g), _NT_DIMS, preferred_element_type=jnp.float32)

    def lane_tiles(a):
        return [a[:, i:i + 128] for i in range(0, a.shape[1], 128)]

    def scores(slot, between):
        q = q_buf[...]
        tiles = []
        for t in range(n_kb):
            keys = pl.ds(t * _KB, _KB)
            k = cache_block(0, slot, t)
            between(t)
            s = lax.dot_general(q, k, _NT_DIMS, preferred_element_type=jnp.float32)
            s_buf[:, keys] = s
            tiles += lane_tiles(s)
        return jnp.max(functools.reduce(jnp.maximum, tiles), axis=-1, keepdims=True)

    def weighted_values(slot, m, between, zero):
        total = pl.ds(pl.multiple_of(sk + zero, dh), dh)
        pending, tiles = [], []
        for t in range(n_kb):
            keys = pl.ds(t * _KB, _KB)
            v = cache_block(1, slot, t)
            between(n_kb + t)
            if len(pending) == 2:
                part = pending.pop(0)
                s_buf[:, total] = part if t == 2 else s_buf[:, total] + part
            p = jnp.exp2(s_buf[:, keys] - m)
            tiles += lane_tiles(p)
            pending.append(jnp.dot(p.astype(v.dtype), v, preferred_element_type=jnp.float32))
        return functools.reduce(jnp.add, pending, s_buf[:, total]), functools.reduce(jnp.add, tiles)

    def head_step(g, burst):
        slot = g & (_SLOTS - 1)
        second = functools.reduce(jnp.logical_and, [g != s for s in skips], g >= 0)
        lane_words = {}

        def issue(block):
            per_block = _BURST // n_kb
            for i in range(block * per_block, (block + 1) * per_block):
                for cache in range(2):
                    n = i + cache * (_BURST - _V_BACK)
                    key = (n // _BURST, n % _LANES, i >= _BURST)
                    if key not in lane_words:
                        word = table[_LANES * burst + (_LANES * key[0] + key[1])]
                        lane_words[key] = jnp.where(second, word, _EMPTY) if key[2] else word
                    word = lane_words[key]
                    for kind in (_PAIR, _SINGLE):
                        pl.when(lax.shift_right_logical(word, _KIND_SHIFT) == kind)(
                            functools.partial(start_load, cache, kind, word, n // _LANES % _DEPTH))

        wait_head(0, g)
        m = scores(slot, issue)
        q_next = project_q(g + 1)
        y = project_out(g - 1, o_buf[...], l_buf[...])
        q_buf[...] = q_next
        acc[...] = jnp.where(((g - 1) & (heads - 1)) == 0, y, acc[...] + y)
        wait_head(1, g)
        o_buf[...], l_buf[...] = weighted_values(slot, m, issue, lax.shift_right_logical(g, 20) * dh)

        @pl.when(jnp.logical_and((g & (heads - 1)) == 0, g > 0))
        def _():
            b = lax.shift_right_logical(jnp.maximum(g - 1, 0), head_bits)
            out_buf[batch_rows(b), :] = acc[...].astype(out_buf.dtype)

        return burst + 1 + second.astype(jnp.int32)

    q_buf[...] = project_q(0)
    acc[...] = jnp.zeros_like(acc)
    o_buf[...] = jnp.zeros_like(o_buf)
    l_buf[...] = jnp.ones_like(l_buf)
    burst = lax.fori_loop(0, n_heads - 1, head_step, issued[0])

    def store(b, sem):
        return pltpu.make_async_copy(out_buf.at[batch_rows(b)], out_hbm.at[batch_rows(b)], sem)

    g = n_heads - 1
    slot = g & (_SLOTS - 1)
    wait_all(kv_buf.at[0, slot], kv_sem.at[0, slot])
    m = scores(slot, lambda block: None)
    wait_all(kv_buf.at[1, slot], kv_sem.at[1, slot])
    for b in range(batch - 1):
        store(b, out_sem.at[0]).start()
    acc[...] += project_out(g - 1, o_buf[...], l_buf[...])
    o, l = weighted_values(slot, m, lambda block: None, lax.shift_right_logical(burst, 20) * dh)
    out_buf[batch_rows(batch - 1), :] = (acc[...] + project_out(g, o, l)).astype(out_buf.dtype)
    last = store(batch - 1, out_sem.at[1])
    last.start()
    wait_all(out_buf.at[pl.ds(0, (batch - 1) * sq)], out_sem.at[0])
    last.wait()


@jax.jit
def pallas_standalone__mha_block_cached__near_ridge_kernel(
    x: jax.Array,
    k_cache: jax.Array,
    v_cache: jax.Array,
    wq: jax.Array,
    wo: jax.Array,
):
    batch, sq, d_model = x.shape
    _, heads, sk, dh = k_cache.shape
    bursts, done, _ = _plan_bursts(batch * heads, sk)
    issued, _ = _plan_issue(bursts, done)

    head_shape = (2, sk // 2, dh)
    w_shape = (2, d_model // 2, heads * dh)
    hbm = pl.BlockSpec(memory_space=pltpu.HBM)
    out = pl.pallas_call(
        functools.partial(_kernel, batch=batch, heads=heads),
        in_specs=[hbm] * 5,
        out_specs=hbm,
        out_shape=jax.ShapeDtypeStruct((batch * sq, d_model), x.dtype),
        scratch_shapes=[
            pltpu.VMEM((batch * sq, d_model), x.dtype),
            pltpu.VMEM(w_shape, wq.dtype),
            pltpu.VMEM(w_shape, wo.dtype),
            pltpu.VMEM((2, _SLOTS) + head_shape, k_cache.dtype),
            pltpu.VMEM((sq, sk + 2 * dh), jnp.float32),
            pltpu.VMEM((sq, dh), x.dtype),
            pltpu.VMEM((sq, dh), jnp.float32),
            pltpu.VMEM((sq, 128), jnp.float32),
            pltpu.VMEM((sq, d_model), jnp.float32),
            pltpu.VMEM((batch * sq, d_model), x.dtype),
            pltpu.SMEM(((issued[-1] + 2) * _LANES,), jnp.int32),
            pltpu.SemaphoreType.DMA((2, _SLOTS)),
            pltpu.SemaphoreType.DMA((3,)),
            pltpu.SemaphoreType.DMA((2,)),
        ],
        compiler_params=pltpu.CompilerParams(
            vmem_limit_bytes=100 * 1024 * 1024,
            disable_bounds_checks=True,
            disable_semaphore_checks=True,
        ),
    )(
        x.reshape(batch * sq, d_model),
        k_cache.reshape((batch * heads,) + head_shape),
        v_cache.reshape((batch * heads,) + head_shape),
        wq.reshape(w_shape),
        wo.T.reshape(w_shape),
    )
    return out.reshape(batch, sq, d_model)
```

```python
import functools

import jax
import jax.numpy as jnp
from jax import lax
import jax.experimental.pallas as pl
import jax.experimental.pallas.tpu as pltpu

_SEG = 32
_LANES = 4
_DEPTH = 4
_BURST = _LANES * _DEPTH
_SLOTS = 16
_KB = 256
_V_BACK = 4
_TAPER = (10, 7, 3)
_COMPUTE_COST = 0.74
_EMPTY, _PAIR, _SINGLE = 0, 1, 2
_KIND_SHIFT, _STEP_SHIFT = 28, 24
_NT_DIMS = (((1,), (1,)), ((), ()))


def _plan_bursts(n_heads, sk):
    n4, n2, n1 = _TAPER
    life = sk // _SEG
    period = life // _LANES
    n_pairs = (n_heads - n4 - n2 - n1) // 2
    assert n_pairs >= _LANES and 2 * n_pairs + n4 + n2 + n1 == n_heads and n4 % 2 == 0
    end4 = n_pairs + n4 // 2
    end2 = end4 + n2
    end1 = end2 + 2 * n1

    def lane(t, a):
        j = t // period - (_LANES - 1) + a
        if j < 0:
            return None
        if j < n_pairs:
            return _PAIR, 2 * j, t % life * _SEG
        row = t % (life // 2) * _SEG
        if a < _LANES // 2:
            return (_SINGLE, 2 * j + 2, row) if j < end4 else None
        if j >= end1 or (j >= end2 and (j - end2) % 2):
            return None
        return _SINGLE, min(max(j + n_pairs, 2 * j - 1), j + end4, (j + end2) // 2 + end4), row

    bursts = []
    t = 0
    while t < period * end1:
        lanes = [lane(t, a) for a in range(_LANES)]
        active = [d for d in lanes if d is not None]
        if len(active) > _LANES // 2 or t < life:
            bursts.append((_SEG, lanes))
            t += _DEPTH
        else:
            rep = _LANES // len(active)
            bursts.append((rep * _SEG, [(k, h, r + i * _SEG) for i in range(rep) for k, h, r in active]))
            t += rep * _DEPTH

    seen = {}
    done = [0] * n_heads
    for b, (step, lanes) in enumerate(bursts):
        for kind, h, row in (d for d in lanes if d is not None):
            for r in range(row, row + _DEPTH * step, step):
                assert r // (sk // 2) == row // (sk // 2) and (kind == _PAIR or r < sk // 2)
                for part in ((h, r), (h + 1, r) if kind == _PAIR else (h, r + sk // 2)):
                    assert part not in seen
                    seen[part] = b
                    done[part[0]] = b + 1
    assert len(seen) == n_heads * life
    return bursts, done, 2 * n_pairs


def _plan_issue(bursts, done, lead=1):
    n_heads = len(done)
    need = [0] * (n_heads + 1)
    for g in reversed(range(n_heads)):
        need[g] = max(done[g] + lead, need[g + 1] - 2)
    issued, skips = [need[0]], []
    now = done[0]
    for g in range(n_heads - 1):
        now = max(now + 2 * _COMPUTE_COST, done[g + 1])
        skip = issued[-1] + 1 >= max(need[g + 1], now + lead) and issued[-1] < len(bursts)
        if skip:
            skips.append(g)
        issued.append(issued[-1] + (1 if skip else 2))
    assert issued[-1] >= len(bursts)
    for g in range(n_heads - 1):
        assert issued[g] >= done[g]
        for _, lanes in bursts[issued[g]:issued[g + 1] + 1]:
            assert all(d is None or d[1] + (d[0] == _PAIR) - _SLOTS < g for d in lanes)
    return issued, skips


def _kernel(x_hbm, k_hbm, v_hbm, wq_hbm, wo_hbm, out_hbm,
            x_buf, wq_buf, wo_buf, kv_buf, s_buf, q_buf, o_buf, l_buf, acc, out_buf,
            table, kv_sem, in_sem, out_sem, *, batch, heads):
    n_heads, _, half_sk, dh = k_hbm.shape
    sk = 2 * half_sk
    half_d = wq_hbm.shape[1]
    sq = x_hbm.shape[0] // batch
    n_kb = sk // _KB
    row_bits = sk.bit_length() - 1
    head_bits = heads.bit_length() - 1
    assert sk == 1 << row_bits and heads == 1 << head_bits
    q_scale = dh ** -0.5

    bursts, done, paired_heads = _plan_bursts(n_heads, sk)
    issued, skips = _plan_issue(bursts, done)

    def encode(step, d):
        if d is None:
            return _EMPTY
        return d[0] << _KIND_SHIFT | step // _SEG << _STEP_SHIFT | d[1] << row_bits | d[2]

    def steady_word(b, a):
        per = sk // _SEG // _BURST
        pair = lax.shift_right_logical(b, per.bit_length() - 1) + (a - (_LANES - 1))
        row = (b & (_LANES * per - 1)) * (_DEPTH * _SEG)
        word = (_PAIR << _KIND_SHIFT | 1 << _STEP_SHIFT) + pair * (2 * sk) + row
        return jnp.where(pair >= 0, word, _EMPTY)

    words = [[encode(step, d) for d in lanes] for step, lanes in bursts]
    words += [[_EMPTY] * _LANES] * (table.shape[0] // _LANES - len(words))
    n_steady = next(b for b, (_, lanes) in enumerate(bursts) if any(d and d[0] == _SINGLE for d in lanes))

    def start_load(cache, kind, word, depth):
        head = lax.shift_right_logical(word & ((1 << _STEP_SHIFT) - 1), row_bits)
        slot = head & (_SLOTS - 1)
        step = lax.shift_right_logical(word, _STEP_SHIFT) & ((1 << _KIND_SHIFT - _STEP_SHIFT) - 1)
        rows = pl.ds(pl.multiple_of((word & (half_sk - 1)) + depth * _SEG * step, _SEG), _SEG)
        if kind == _PAIR:
            half = lax.shift_right_logical(word, row_bits - 1) & 1
            src = (k_hbm, v_hbm)[cache].at[pl.ds(head, 2), half, rows]
            dst = kv_buf.at[cache, pl.ds(slot, 2), half, rows]
        else:
            src = (k_hbm, v_hbm)[cache].at[head, :, rows]
            dst = kv_buf.at[cache, slot, :, rows]
        pltpu.make_async_copy(src, dst, kv_sem.at[cache, slot]).start(priority=cache)

    def wait_all(buf, sem):
        pltpu.make_async_copy(buf, buf, sem).wait()

    def wait_head(cache, g):
        slot = g & (_SLOTS - 1)

        @pl.when(jnp.logical_and(g < paired_heads, (g & 1) == 0))
        def _():
            wait_all(kv_buf.at[cache, pl.ds(slot, 2)], kv_sem.at[cache, slot])

        @pl.when(g >= paired_heads)
        def _():
            wait_all(kv_buf.at[cache, slot], kv_sem.at[cache, slot])

    x_rows = 32
    n_x = batch * sq // x_rows
    x_first = n_x // 4 * 2 - 2
    assert n_x * x_rows == batch * sq and n_x % 2 == 0

    def start_x(j, priority):
        rows = pl.ds(pl.multiple_of(j * x_rows, x_rows), x_rows)
        pltpu.make_async_copy(x_hbm.at[rows], x_buf.at[rows], in_sem.at[2]).start(priority=priority)

    w_cols = 1024
    w_tiles = half_d // _LANES // 8
    assert w_tiles * _LANES * 8 == half_d

    def fill_table(b, _):
        for a in range(_LANES):
            table[_LANES * b + a] = steady_word(b, a)
        return 0

    def start_weights(j, _):
        for c in range(0, heads * dh, w_cols):
            for a in range(_LANES):
                idx = (slice(None), pl.ds(pl.multiple_of((j + a * w_tiles) * 8, 8), 8), pl.ds(c, w_cols))
                for i, (src, dst) in enumerate(((wq_hbm, wq_buf), (wo_hbm, wo_buf))):
                    pltpu.make_async_copy(src.at[idx], dst.at[idx], in_sem.at[i]).start(priority=i)
        share = pl.cdiv(n_steady, w_tiles)
        return lax.fori_loop(j * share, jnp.minimum((j + 1) * share, n_steady), fill_table, 0)

    def start_x_rest(j, _):
        for half in range(2):
            start_x(x_first + j + half * ((n_x - x_first) // 2), half)
        return 0

    def start_first_bursts(b, _):
        for depth in range(_DEPTH):
            for a in range(_LANES):
                for cache in range(2):
                    word = table[_LANES * (b if cache else jnp.maximum(b - 1, 0)) + a]
                    live = word != _EMPTY
                    if cache == 0:
                        live = jnp.logical_and(live, b >= 1)
                    elif depth * _LANES >= _BURST - _V_BACK:
                        live = jnp.logical_and(live, b < issued[0])
                    pl.when(live)(functools.partial(start_load, cache, _PAIR, word, depth))
        return 0

    for j in range(x_first):
        start_x(j, 1)
    lax.fori_loop(0, w_tiles, start_weights, 0)
    lax.fori_loop(0, (n_x - x_first) // 2, start_x_rest, 0)
    assert issued[0] + 1 <= n_steady
    lax.fori_loop(0, issued[0] + 1, start_first_bursts, 0)
    for b in range(n_steady, len(words)):
        for a in range(_LANES):
            table[_LANES * b + a] = jnp.int32(words[b][a])
    for i, buf in enumerate((wq_buf, wo_buf, x_buf)):
        wait_all(buf, in_sem.at[i])

    def head_weights(w_buf, g):
        h = g & (heads - 1)
        cols = pl.ds(h * dh if isinstance(h, int) else pl.multiple_of(h * dh, dh), dh)
        return w_buf[:, :, cols].reshape(2 * half_d, dh)

    def cache_block(cache, slot, t):
        return kv_buf[cache, slot, t * _KB // half_sk, pl.ds(t * _KB % half_sk, _KB), :]

    def batch_rows(b):
        return pl.ds(b * sq if isinstance(b, int) else pl.multiple_of(b * sq, 16), sq)

    def project_q(g):
        b = g >> head_bits if isinstance(g, int) else lax.shift_right_logical(g, head_bits)
        q = jnp.dot(x_buf[batch_rows(b), :], head_weights(wq_buf, g), preferred_element_type=jnp.float32)
        return (q * q_scale).astype(q_buf.dtype)

    def project_out(g, o, l):
        o = (o * (1.0 / jnp.sum(l, axis=-1, keepdims=True))).astype(wo_buf.dtype)
        return lax.dot_general(o, head_weights(wo_buf, g), _NT_DIMS, preferred_element_type=jnp.float32)

    def lane_tiles(a):
        return [a[:, i:i + 128] for i in range(0, a.shape[1], 128)]

    def scores(g, slot, between):
        q = q_buf[g]
        tiles = []
        for t in range(n_kb):
            keys = pl.ds(t * _KB, _KB)
            k = cache_block(0, slot, t)
            between(t)
            s = lax.dot_general(q, k, _NT_DIMS, preferred_element_type=jnp.float32)
            s_buf[:, keys] = s
            tiles += lane_tiles(s)
        return jnp.max(functools.reduce(jnp.maximum, tiles), axis=-1, keepdims=True)

    def weighted_values(slot, m, between, zero):
        total = pl.ds(pl.multiple_of(sk + zero, dh), dh)
        pending, tiles = [], []
        for t in range(n_kb):
            keys = pl.ds(t * _KB, _KB)
            v = cache_block(1, slot, t)
            between(n_kb + t)
            if len(pending) == 2:
                part = pending.pop(0)
                s_buf[:, total] = part if t == 2 else s_buf[:, total] + part
            p = jnp.exp(s_buf[:, keys] - m)
            tiles += lane_tiles(p)
            pending.append(jnp.dot(p.astype(v.dtype), v, preferred_element_type=jnp.float32))
        return functools.reduce(jnp.add, pending, s_buf[:, total]), functools.reduce(jnp.add, tiles)

    def head_step(g, burst, project):
        slot = g & (_SLOTS - 1)
        second = functools.reduce(jnp.logical_and, [g != s for s in skips], g >= 0)
        lane_words = {}

        def issue(block):
            per_block = _BURST // n_kb
            for i in range(block * per_block, (block + 1) * per_block):
                for cache in range(2):
                    n = i + cache * (_BURST - _V_BACK)
                    key = (n // _BURST, n % _LANES, i >= _BURST)
                    if key not in lane_words:
                        word = table[_LANES * burst + (_LANES * key[0] + key[1])]
                        lane_words[key] = jnp.where(second, word, _EMPTY) if key[2] else word
                    word = lane_words[key]
                    for kind in (_PAIR, _SINGLE):
                        pl.when(lax.shift_right_logical(word, _KIND_SHIFT) == kind)(
                            functools.partial(start_load, cache, kind, word, n // _LANES % _DEPTH))

        wait_head(0, g)
        m = scores(g, slot, issue)
        if project:
            for i in (2, 3):
                q_buf[2 * g + i] = project_q(2 * g + i)
        y = project_out(g - 1, o_buf[...], l_buf[...])
        acc[...] = jnp.where(((g - 1) & (heads - 1)) == 0, y, acc[...] + y)
        wait_head(1, g)
        o_buf[...], l_buf[...] = weighted_values(slot, m, issue, lax.shift_right_logical(g, 20) * dh)

        @pl.when(jnp.logical_and((g & (heads - 1)) == 0, g > 0))
        def _():
            b = lax.shift_right_logical(jnp.maximum(g - 1, 0), head_bits)
            out_buf[batch_rows(b), :] = acc[...].astype(out_buf.dtype)

        return burst + 1 + second.astype(jnp.int32)

    for g in range(2):
        q_buf[g] = project_q(g)
    acc[...] = jnp.zeros_like(acc)
    o_buf[...] = jnp.zeros_like(o_buf)
    l_buf[...] = jnp.ones_like(l_buf)
    split = n_heads // 2 - 1
    burst = lax.fori_loop(0, split, functools.partial(head_step, project=True), issued[0])
    burst = lax.fori_loop(split, n_heads - 1, functools.partial(head_step, project=False), burst)

    def store(b, sem):
        return pltpu.make_async_copy(out_buf.at[batch_rows(b)], out_hbm.at[batch_rows(b)], sem)

    g = n_heads - 1
    slot = g & (_SLOTS - 1)
    wait_all(kv_buf.at[0, slot], kv_sem.at[0, slot])
    m = scores(g, slot, lambda block: None)
    wait_all(kv_buf.at[1, slot], kv_sem.at[1, slot])
    for b in range(batch - 1):
        store(b, out_sem.at[0]).start()
    acc[...] += project_out(g - 1, o_buf[...], l_buf[...])
    o, l = weighted_values(slot, m, lambda block: None, lax.shift_right_logical(burst, 20) * dh)
    out_buf[batch_rows(batch - 1), :] = (acc[...] + project_out(g, o, l)).astype(out_buf.dtype)
    last = store(batch - 1, out_sem.at[1])
    last.start()
    wait_all(out_buf.at[pl.ds(0, (batch - 1) * sq)], out_sem.at[0])
    last.wait()


@jax.jit
def pallas_standalone__mha_block_cached__near_ridge_kernel(
    x: jax.Array,
    k_cache: jax.Array,
    v_cache: jax.Array,
    wq: jax.Array,
    wo: jax.Array,
):
    batch, sq, d_model = x.shape
    _, heads, sk, dh = k_cache.shape
    bursts, done, _ = _plan_bursts(batch * heads, sk)
    issued, _ = _plan_issue(bursts, done)

    head_shape = (2, sk // 2, dh)
    w_shape = (2, d_model // 2, heads * dh)
    hbm = pl.BlockSpec(memory_space=pltpu.HBM)
    out = pl.pallas_call(
        functools.partial(_kernel, batch=batch, heads=heads),
        in_specs=[hbm] * 5,
        out_specs=hbm,
        out_shape=jax.ShapeDtypeStruct((batch * sq, d_model), x.dtype),
        scratch_shapes=[
            pltpu.VMEM((batch * sq, d_model), x.dtype),
            pltpu.VMEM(w_shape, wq.dtype),
            pltpu.VMEM(w_shape, wo.dtype),
            pltpu.VMEM((2, _SLOTS) + head_shape, k_cache.dtype),
            pltpu.VMEM((sq, sk + 2 * dh), jnp.float32),
            pltpu.VMEM((batch * heads, sq, dh), x.dtype),
            pltpu.VMEM((sq, dh), jnp.float32),
            pltpu.VMEM((sq, 128), jnp.float32),
            pltpu.VMEM((sq, d_model), jnp.float32),
            pltpu.VMEM((batch * sq, d_model), x.dtype),
            pltpu.SMEM(((issued[-1] + 2) * _LANES,), jnp.int32),
            pltpu.SemaphoreType.DMA((2, _SLOTS)),
            pltpu.SemaphoreType.DMA((3,)),
            pltpu.SemaphoreType.DMA((2,)),
        ],
        compiler_params=pltpu.CompilerParams(
            vmem_limit_bytes=100 * 1024 * 1024,
            disable_bounds_checks=True,
            disable_semaphore_checks=True,
        ),
    )(
        x.reshape(batch * sq, d_model),
        k_cache.reshape((batch * heads,) + head_shape),
        v_cache.reshape((batch * heads,) + head_shape),
        wq.reshape(w_shape),
        wo.T.reshape(w_shape),
    )
    return out.reshape(batch, sq, d_model)
```
